```python
import os as _os
_os.environ.setdefault("JAX_PLATFORMS", "cpu")
import jax
import jax.numpy as jnp

def _softmax(x, axis=-1):
    return jax.nn.softmax(x, axis=axis)
def _gelu(x):
    return jax.nn.gelu(x, approximate=True)
def _silu(x):
    return jax.nn.silu(x)
def _sigmoid(x):
    return jax.nn.sigmoid(x)
def _layernorm(x, axis=-1, eps=1e-5):
    m = jnp.mean(x, axis=axis, keepdims=True)
    v = jnp.var(x, axis=axis, keepdims=True)
    return (x - m) / jnp.sqrt(v + eps)
def _scatter_add(tgt, idx, src, axis=0):
    return tgt.at[idx].add(src)
def _segment_sum(src, seg, n):
    return jax.ops.segment_sum(src, seg, n)
class _Rng:
    def __init__(self, key):
        self._k = key
    def _next(self):
        self._k, sub = jax.random.split(self._k)
        return sub
    def normal(self, shape):
        return jax.random.normal(self._next(), shape, dtype=jnp.bfloat16)
    def randint(self, lo, hi, shape):
        return jax.random.randint(self._next(), shape, lo, hi, dtype=jnp.int32)
    def uniform(self, shape, lo=0.0, hi=1.0):
        return jax.random.uniform(self._next(), shape, jnp.bfloat16, lo, hi)
    def permutation(self, n):
        return jax.random.permutation(self._next(), n)


kernel_name = 'standalone__mixer_token_mlp__sampling'

def setup_inputs():
    _rng = _Rng(jax.random.key(int.from_bytes(__import__("os").urandom(4), "little")))
    _w = (lambda a: (lambda t: t.astype(jnp.bfloat16) if jnp.issubdtype(t.dtype, jnp.floating) else t)(jnp.asarray(a)))
    B, S, D, F = 32, 16, 1024, 3584
    return {
        "x": _w((lambda *s: _rng.normal(s) * 0.05)(B, S, D)),
        "w1": _w((lambda *s: _rng.normal(s) * 0.05)(S, F) * (S ** -0.5)),
        "b1": _w((lambda *s: _rng.normal(s) * 0.05)(F) * 0.02),
        "w2": _w((lambda *s: _rng.normal(s) * 0.05)(F, S) * (F ** -0.5)),
        "b2": _w((lambda *s: _rng.normal(s) * 0.05)(S) * 0.02),
    }

def reference(x, w1, b1, w2, b2):
    B, S, D = x.shape
    h = _layernorm(x, axis=-1)
    u = jnp.einsum("bsd,sf->bdf", h, w1) + b1
    u = _gelu(u)
    y = jnp.einsum("bdf,fs->bds", u, w2) + b2
    return (lambda x, *d: x.transpose(*d))(y, 0, 2, 1)
```

```python
import functools
import numpy as np
import jax, jax.numpy as jnp
from jax import lax
from jax.experimental import pallas as pl
from jax.experimental.pallas import tpu as pltpu

C1 = float(np.sqrt(2.0 / np.pi))
C2 = 0.044715 * C1
ALPHA = C2 ** (1.0 / 3.0)
KAPPA = C1 / ALPHA
A_HI = float(np.float32(ALPHA).astype(jnp.bfloat16).astype(np.float32))
f32, bf16 = jnp.float32, jnp.bfloat16
NN = (((1,), (0,)), ((), ()))
NT = (((1,), (1,)), ((), ()))

def make(fc=256, pat=(16,), dc=512, lag=1, gf32=True, nb=1, flags=None, strassen=False, bload=True, order='mav', lin=True, lnpos=2, mpos=0):
    S, L = 16, 128
    F = 3584
    nit = F // fc
    nvs = [pat[i % len(pat)] for i in range(nit)]
    goff = np.concatenate([[0], np.cumsum(nvs)]) // 16
    npair = int(goff[-1])
    NW = 58 if strassen else 34
    NH = 7 if strassen else 4

    def layernorm(x, ha_ref, hv_ref, slot):
        x = x.astype(f32)
        D = x.shape[1]
        m = jnp.mean(x, axis=-1, keepdims=True)
        xc = x - m
        v = jnp.mean(xc * xc, axis=-1, keepdims=True)
        h = (xc * (ALPHA * lax.rsqrt(v + 1e-5))).astype(bf16)
        ha_ref[slot] = h
        if npair:
            hr = h.astype(f32)
            for p in range(D // (2 * L)):
                b11, b12 = hr[:8, 2 * p * L:(2 * p + 1) * L], hr[:8, (2 * p + 1) * L:(2 * p + 2) * L]
                b21, b22 = hr[8:, 2 * p * L:(2 * p + 1) * L], hr[8:, (2 * p + 1) * L:(2 * p + 2) * L]
                if strassen:
                    t1 = b12 - b11; t2 = b22 - t1
                    hs = [b11, b21, b22, b21 - t2, t1, t2, b22 - b12]
                else:
                    hs = [b11, b21, b12, b22]
                for k, t in enumerate(hs):
                    if bload:
                        hv_ref[slot, p, k] = t
                    else:
                        for s in range(8):
                            hv_ref[slot, p, k * 8 + s] = jnp.broadcast_to(t[s:s + 1], (8, L))

    def kern(x0_ref, xn_ref, w1_ref, b1_ref, w2t_ref, b2_ref, o_ref, w1t_s, w2t_s, m_s, c_s, wb_s, ha_s, hv_s):
        D = x0_ref.shape[-1]
        step = pl.program_id(0)

        @pl.when(step == 0)
        def _():
            row = lax.broadcasted_iota(jnp.int32, (S, L), 0)
            b1 = b1_ref[...].astype(f32)
            macc = jnp.zeros((S, L), f32)
            for j in range(F // L):
                ext = jnp.where(row < 2, b1[j:j + 1, :], 0.0).astype(bf16)
                wj = w1_ref[:, j * L:(j + 1) * L]
                blk = jnp.concatenate([wj, ext, wj, jnp.zeros((L - 3 * S, L), bf16)], axis=0)
                wt = blk.T
                w1t_s[j * L:(j + 1) * L, :] = wt
                w2j = w2t_ref[:, j * L:(j + 1) * L]
                w2t_s[:, j * L:(j + 1) * L] = w2j
                macc = macc + lax.dot_general(w2j, wt, NN, preferred_element_type=f32)
            col = lax.broadcasted_iota(jnp.int32, (S, L), 1)
            mhi = macc.astype(bf16).astype(f32)
            m_s[...] = jnp.where(col < S, mhi, jnp.where(col < 2 * S, 0.0, macc - mhi)).astype(bf16)
            b2 = jnp.sum(jnp.where(lax.broadcasted_iota(jnp.int32, (S, S), 0) == lax.broadcasted_iota(jnp.int32, (S, S), 1),
                                   b2_ref[...].astype(f32), 0.0), axis=1, keepdims=True)
            c_s[...] = jnp.broadcast_to((0.5 * macc[:, S:S + 1] if lin else 0.0) + b2, (S, L))
            for i in range(nit):
                for q in range(nvs[i] // 16):
                    r0 = (i + 1) * fc - nvs[i] + 16 * q
                    w = w1t_s[r0:r0 + 16, :].astype(f32)
                    bc = lambda r, c: jnp.broadcast_to(w[8 * r:8 * r + 8, c:c + 1], (8, L))
                    pi = goff[i] + q
                    for s in range(8):
                        a11, a12, a21, a22 = bc(0, s), bc(0, 8 + s), bc(1, s), bc(1, 8 + s)
                        if strassen:
                            s1 = a21 + a22; s2 = s1 - a11
                            ws = [a11, a12, a12 - s2, a22, s1, s2, a11 - a21]
                        else:
                            ws = [a11, a12, a21, a22]
                        for k, t in enumerate(ws):
                            wb_s[pi, k * 8 + s] = t
                    c1, c2 = ALPHA * bc(0, S), ALPHA * bc(1, S)
                    wb_s[pi, NW - 2] = c1
                    wb_s[pi, NW - 1] = c2 - c1 if strassen else c2
            for b in range(nb):
                layernorm(x0_ref[b], ha_s, hv_s, b)

        cur = (step % 2) * nb
        nxt = nb - cur
        row = lax.broadcasted_iota(jnp.int32, (S, dc), 0)
        ext = jnp.where(row == 0, A_HI, jnp.where(row == 1, ALPHA - A_HI, 0.0)).astype(bf16)

        def act(u):
            t = jnp.tanh(u * (u * u + KAPPA))
            return u * t if lin else u * t + u

        def vpu_part(b, d0, i):
            rows = []
            for q in range(nvs[i] // 16):
                pi = goff[i] + q
                top, bot = [], []
                for p in range(d0 // (2 * L), (d0 + dc) // (2 * L)):
                    def hb(k, s):
                        if bload:
                            return jnp.broadcast_to(hv_s[cur + b, p, k, s:s + 1, :], (8, L))
                        return hv_s[cur + b, p, k * 8 + s]
                    def mac(a, kw, kh):
                        for s in range(8):
                            t = wb_s[pi, kw * 8 + s] * hb(kh, s)
                            a = t if a is None else a + t
                        return a
                    c1, c2 = wb_s[pi, NW - 2], wb_s[pi, NW - 1]
                    if strassen:
                        p1 = mac(c1, 0, 0)
                        p5 = mac(None, 4, 4)
                        c11 = mac(p1, 1, 1)
                        u2 = mac(p1, 5, 5)
                        c12 = mac(u2 + p5, 2, 2)
                        u3 = mac(u2 + c2, 6, 6)
                        c21 = mac(u3, 3, 3)
                        c22 = u3 + p5
                    else:
                        c11 = mac(mac(c1, 0, 0), 1, 1); c12 = mac(mac(c1, 0, 2), 1, 3)
                        c21 = mac(mac(c2, 2, 0), 3, 1); c22 = mac(mac(c2, 2, 2), 3, 3)
                    top += [c11, c12]; bot += [c21, c22]
                rows += [jnp.concatenate(top, axis=1), jnp.concatenate(bot, axis=1)]
            return jnp.concatenate(rows, axis=0)

        items = [(b, d0, i) for b in range(nb) for d0 in range(0, D, dc) for i in range(nit)]
        gs, acc, ylin = {}, {}, {}
        for n in range(len(items) + lag):
            st = {}
            def do_m():
                b, d0, i = items[n]
                h = ha_s[cur + b, :, d0:d0 + dc]
                w = w1t_s[i * fc:(i + 1) * fc - nvs[i], :2 * S]
                st['u'] = lax.dot_general(w, jnp.concatenate([h, ext], axis=0), NN, preferred_element_type=f32)
                if lin and i == mpos:
                    ylin[(b, d0)] = lax.dot_general(m_s[:, :3 * S], jnp.concatenate([h, ext, h], axis=0), NN, preferred_element_type=f32)
            def do_a():
                st['g'] = act(st['u'])
            def do_v():
                b, d0, i = items[n]
                if nvs[i]:
                    st['gv'] = act(vpu_part(b, d0, i))
            def do_y():
                j = n - lag
                if j < 0: return
                b, d0, i = items[j]
                y = lax.dot_general(w2t_s[:, i * fc:(i + 1) * fc], gs.pop(j), NN, preferred_element_type=f32)
                acc[(b, d0)] = y if i == 0 else acc[(b, d0)] + y
                if i == nit - 1:
                    a = acc.pop((b, d0))
                    if lin: a = a + ylin.pop((b, d0))
                    c = jnp.concatenate([c_s[...]] * (dc // L), axis=1)
                    o_ref[b, :, d0:d0 + dc] = (a * (0.5 / ALPHA) + c).astype(o_ref.dtype)
            for ch in (order if 'y' in order else order + 'y'):
                if ch == 'y': do_y()
                elif n < len(items): {'m': do_m, 'a': do_a, 'v': do_v}[ch]()
            if n < len(items):
                g = jnp.concatenate([st['g'], st['gv']], axis=0) if 'gv' in st else st['g']
                gs[n] = g if gf32 else g.astype(bf16)
                b, d0, i = items[n]
                if d0 == 0 and i == lnpos:
                    layernorm(xn_ref[b], ha_s, hv_s, nxt + b)

    @jax.jit
    def fn(x, w1, b1, w2, b2):
        B, S, D = x.shape
        ns = B // nb
        return pl.pallas_call(
            kern, grid=(ns,),
            in_specs=[pl.BlockSpec((nb, S, D), lambda b: (0, 0, 0)),
                      pl.BlockSpec((nb, S, D), lambda b: (jnp.minimum(b + 1, ns - 1), 0, 0)),
                      pl.BlockSpec((S, F), lambda b: (0, 0)),
                      pl.BlockSpec((F // L, L), lambda b: (0, 0)),
                      pl.BlockSpec((S, F), lambda b: (0, 0)),
                      pl.BlockSpec((1, S), lambda b: (0, 0))],
            out_specs=pl.BlockSpec((nb, S, D), lambda b: (b, 0, 0)),
            out_shape=jax.ShapeDtypeStruct((B, S, D), x.dtype),
            scratch_shapes=[pltpu.VMEM((F, L), bf16), pltpu.VMEM((S, F), bf16), pltpu.VMEM((S, L), bf16), pltpu.VMEM((S, L), f32),
                            pltpu.VMEM((max(npair, 1), NW, 8, L), f32), pltpu.VMEM((2 * nb, S, D), bf16),
                            pltpu.VMEM((2 * nb, D // (2 * L), NH if bload else NH * 8, 8, L), f32)],
            compiler_params=pltpu.CompilerParams(dimension_semantics=("arbitrary",), vmem_limit_bytes=100 * 2**20, flags=flags),
            name="mixer",
        )(x, x, w1, b1.reshape(F // L, L), w2.T, b2.reshape(1, S))
    return fn


_fn = make()


@jax.jit
def pallas_standalone__mixer_token_mlp__sampling_kernel(x, w1, b1, w2, b2):
    return _fn(x, w1, b1, w2, b2)
```

```python
import jax
import jax.numpy as jnp
import numpy as np
from jax import lax
from jax.experimental import pallas as pl
from jax.experimental.pallas import tpu as pltpu

_C1 = float(np.sqrt(2.0 / np.pi))
ALPHA = (0.044715 * _C1) ** (1.0 / 3.0)
KAPPA = _C1 / ALPHA
ALPHA_HI = float((np.float32(ALPHA).view(np.uint32) & np.uint32(0xFFFF0000)).view(np.float32))
LN_EPS = 1e-5

LANES = 128
BLK = 16
WIDTH = 2 * LANES
STREAMS = 2
LAG = 8
NPROD = 7 * 8

f32, bf16, i32 = jnp.float32, jnp.bfloat16, jnp.int32

CFG = dict(
    step=4,
    mxu_only=(5, 11, 16, 22, 27),
    warmup=(0, 1, 2),
    cooldown=(),
    spread=(8, 10, 12, 14, 16, 18, 20),
    act=7,
    group=4,
    mxu_cols=14,
    ln_at=14,
    order=0,
    swap=1,
    ln_tie=1,
    osplit=1,
    hm=8,
    dma=0,
)


def _dot(a, b):
    return lax.dot_general(a, b, (((1,), (0,)), ((), ())), preferred_element_type=f32)


def _words(a):
    return pltpu.bitcast(a, i32)


def _bf16(words):
    return pltpu.bitcast(words, bf16)


def _act(v):
    return v * jnp.tanh(v * (v * v + KAPPA))


def _plan(ntile, nbatch, d, cfg):
    passes = [(b, d0) for b in range(nbatch) for d0 in range(0, d, STREAMS * WIDTH)]

    def on_mxu(p, j):
        full = (j in cfg["mxu_only"] or (p == 0 and j in cfg["warmup"])
                or (p == len(passes) - 1 and j in cfg["cooldown"]))
        return [(j, r) for r in range(7 if full else 6, -1, -1)]

    events = []
    for k in range(STREAMS):
        blocks, tiles = [], []
        for p, (b, d0) in enumerate(passes):
            where = (b, d0 + k * WIDTH)
            blocks.append((where, (ntile, 0)))
            for j in range(ntile):
                blocks += [(where, blk) for blk in on_mxu(p, j)]
                tiles.append((where, j, len(blocks) + LAG))
        cuts = sorted({0, len(tiles), *range((k + cfg["swap"]) % 2, len(tiles), 2)})
        due = {tiles[hi - 1][2]: tiles[lo:hi] for lo, hi in zip(cuts, cuts[1:])}
        carried = [blk for _, blk in blocks[:LAG]]
        time, run = 0, []
        for i in range(LAG, len(blocks) + LAG + 1):
            if run and (i in due or i == len(blocks) or blocks[i][0] != run[0][0]):
                events.append((time, k, ("v", *run[0][0], [blk for _, blk in run])))
                time, run = time + len(run), []
            for where in sorted({t[0] for t in due.get(i, [])}):
                js = [t[1] for t in due[i] if t[0] == where]
                events.append((time, k, ("y", *where, js)))
                time += len(js)
            if i < len(blocks):
                run.append(blocks[i])
            elif i == len(blocks):
                events.append((time, k, ("carry", k * WIDTH)))
                time += LAG
    events = [e[2] for e in sorted(events, key=lambda e: e[:2])]
    kinds = [e[0] for e in events]
    assert "v" not in kinds[kinds.index("carry"):]
    return carried, events


def _kernel(cfg, x_hbm, w1_hbm, b1_hbm, w2t_hbm, b2_hbm, o_hbm,
            w1_in, b1_in, w2t_in, b2_in, x_ref, o_ref, sems,
            w1t_ref, w2t_ref, const_ref, wv_ref, carry_ref, *h_refs):
    B, S, D = x_ref.shape
    ntile = w1_in.shape[1] // LANES
    nb = cfg["step"]
    pitch = max(8, cfg["hm"])
    h_refs, hv_refs = h_refs[:nb], h_refs[nb:]
    vpu_tiles = [j for j in range(ntile) if j not in cfg["mxu_only"]]
    carried, events = _plan(ntile, nb, D, cfg)

    def iota(shape, axis):
        return lax.broadcasted_iota(i32, shape, axis)

    def layernorm(first):
        x = x_ref[pl.ds(first, nb)].astype(f32)
        xc = x - jnp.sum(x, axis=-1, keepdims=True) * (1.0 / D)
        var = jnp.sum(xc * xc, axis=-1, keepdims=True) * (1.0 / D)
        h = (xc * (ALPHA * lax.rsqrt(var + LN_EPS))).astype(bf16)
        for b in range(nb):
            h_refs[b][:8] = _words(h[b])
        return var

    def hidden_mxu(b, d0, blocks):
        h = _bf16(h_refs[b][:8, d0:d0 + WIDTH])
        row = iota((S, WIDTH), 0)
        one = jnp.where(row == 0, ALPHA_HI, jnp.where(row == 1, ALPHA - ALPHA_HI, 0.0)).astype(bf16)
        w = _bf16(jnp.concatenate([w1t_ref[pl.ds(8 * (8 * j + r), 8), :] for j, r in blocks], axis=0))
        assert blocks[0][0] != ntile or all(j < 3 for j, _ in blocks[1:])
        rhs = [h, one, h] if blocks[0][0] == ntile else [h, one]
        return _dot(w[:, :S * len(rhs)], jnp.concatenate(rhs, axis=0))

    def write_carry(d0):
        v = hidden_mxu(0, d0, carried)
        for i in range(LAG):
            vi = v[BLK * i:BLK * (i + 1)]
            carry_ref[BLK * i:BLK * (i + 1), d0:d0 + WIDTH] = _act(vi) if 0 < i <= cfg["act"] else vi

    def write_vpu_operand(b, d0, lo, hi):
        h = _bf16(h_refs[b][:8, d0:d0 + WIDTH]).astype(f32)
        h11, h12, h21, h22 = h[:8, :LANES], h[:8, LANES:], h[8:, :LANES], h[8:, LANES:]
        t1 = h12 - h11
        t2 = h22 - t1
        rows = jnp.concatenate([h11, h21, h22, h21 - t2, t1, t2, h22 - h12][lo:hi], axis=0)
        ref = hv_refs[(b * D + d0) // WIDTH]
        if cfg["hm"] == 1 and hi - lo == 1:
            ref[pl.ds(64 * lo, 64), :] = jnp.broadcast_to(rows[:, None, :], (8, 8, LANES)).reshape(64, LANES)
            return ref
        for r in range(8):
            ref[pl.ds(8 * pitch * lo + r, 8 * (hi - lo), stride=pitch), :] = rows
        return ref

    def hidden_vpu(b, d0, j):
        i, ref = vpu_tiles.index(j), hv_refs[(b * D + d0) // WIDTH]

        def mac(acc, k):
            for n in range(8 * k, 8 * k + 8):
                term = wv_ref[i, n] * ref[pl.ds(pitch * n, 8), :]
                acc = term if acc is None else acc + term
            return acc

        if cfg["order"] == 1:
            p5 = mac(None, 4)
        u1 = mac(wv_ref[i, NPROD], 0)
        if cfg["order"] == 2:
            c11 = mac(u1, 1)
        u2 = mac(u1, 5)
        u3 = mac(u2 + wv_ref[i, NPROD + 1], 6)
        if cfg["order"] != 1:
            p5 = mac(None, 4)
        if cfg["order"] != 2:
            c11 = mac(u1, 1)
        c12 = mac(p5, 2) + u2 if cfg["order"] == 3 else mac(u2 + p5, 2)
        top = jnp.concatenate([c11, c12], axis=1)
        bottom = jnp.concatenate([mac(u3, 3), u3 + p5], axis=1)
        return jnp.concatenate([top, bottom], axis=0)

    def write_vpu_weights(w, first):
        n = w.shape[0] // BLK
        pick = jnp.concatenate([iota((2 * S, LANES), 0) == c for c in range(cfg["mxu_cols"])], axis=1)
        picked = _dot(w[:, :2 * S], pick.astype(bf16))

        def column(c):
            if c < cfg["mxu_cols"]:
                col = picked[:, c * LANES:(c + 1) * LANES]
            else:
                col = jnp.broadcast_to(w.astype(f32)[:, c:c + 1], (BLK * n, LANES))
            col = col.reshape(n, 2, 8, LANES)
            return col[:, 0], col[:, 1]

        for s in range(8):
            (w11, w21), (w12, w22) = column(s), column(8 + s)
            s1 = w21 + w22
            s2 = s1 - w11
            for k, t in enumerate([w11, w12, w12 - s2, w22, s1, s2, w11 - w21]):
                wv_ref[first:first + n, 8 * k + s] = t
        bias1, bias2 = column(S)
        wv_ref[first:first + n, NPROD] = ALPHA * bias1
        wv_ref[first:first + n, NPROD + 1] = ALPHA * (bias2 - bias1)

    def output_copy(first, n):
        rows = pl.ds(first, n)
        return pltpu.make_async_copy(o_ref.at[rows], o_hbm.at[rows], sems.at[2])

    copies = [pltpu.make_async_copy(src, dst, sems.at[0]) for src, dst in [
        (w1_hbm, w1_in), (b1_hbm, b1_in), (w2t_hbm, w2t_in), (b2_hbm, b2_in),
        (x_hbm.at[:nb], x_ref.at[:nb])]]
    rest_of_x = pltpu.make_async_copy(x_hbm.at[nb:], x_ref.at[nb:], sems.at[1])
    for copy in copies:
        copy.start()
    if cfg["dma"] == 2:
        rest_of_x = pltpu.make_async_copy(x_hbm.at[nb:2 * nb], x_ref.at[nb:2 * nb], sems.at[0])
        late_x = pltpu.make_async_copy(x_hbm.at[2 * nb:], x_ref.at[2 * nb:], sems.at[1])
    if cfg["dma"] == 0:
        rest_of_x.start()
    for copy in copies:
        copy.wait()
    if cfg["dma"]:
        rest_of_x.start()
    if cfg["dma"] == 2:
        late_x.start()

    b1 = b1_in[...].astype(f32).reshape(ntile, LANES)
    w21 = jnp.zeros((S, LANES), f32)
    pending = []
    for j in range(ntile):
        cols = slice(j * LANES, (j + 1) * LANES)
        w1, w2t = w1_in[:, cols], w2t_in[:, cols]
        bias = jnp.where(iota((S, LANES), 0) < 2, b1[j:j + 1], 0.0).astype(bf16)
        wt = jnp.concatenate([w1, bias, w1, jnp.zeros((LANES - 3 * S, LANES), bf16)], axis=0).T
        w1t_ref[pl.ds(64 * j, 64), :] = jnp.where(iota((64, LANES), 1) < 2 * S, _words(wt), 0) if j < 3 else _words(wt)
        w2t_ref[:8, cols] = _words(w2t)
        w21 = w21 + _dot(w2t, wt)
        if j in vpu_tiles:
            pending.append(wt[LANES - BLK:])
        if j == cfg["ln_at"]:
            layernorm(0)
        if pending and (j == 0 or (j + 1) % cfg["group"] == 0 or j == ntile - 1):
            write_vpu_weights(jnp.concatenate(pending, axis=0), sum(t <= j for t in vpu_tiles) - len(pending))
            pending = []
    lane, head = iota((S, LANES), 1), w21.astype(bf16).astype(f32)
    w1t_ref[pl.ds(64 * ntile, 8), :] = _words(
        jnp.where(lane < S, head, jnp.where(lane < 2 * S, 0.0, w21 - head)).astype(bf16))
    b2 = jnp.where(iota((S, S), 0) == iota((S, S), 1), b2_in[...].astype(f32)[None, :], 0.0)
    const_ref[...] = jnp.broadcast_to(
        ALPHA * w21[:, S:S + 1] + (2 * ALPHA) * jnp.sum(b2, axis=1, keepdims=True), (S, LANES))
    for k in range(STREAMS):
        write_carry(k * WIDTH)
    rest_of_x.wait()

    @pl.loop(0, B // nb)
    def _(it):
        if cfg["dma"] == 2:
            pl.when(it == 1)(late_x.wait)
        zero = pl.multiple_of((it >> 20) * 8, 8)

        def order_loads_after(ref, value):
            ref[pl.ds(ref.shape[0] - 8 + zero, 8), :LANES] = pltpu.bitcast(value, ref.dtype)

        def start(linear):
            return jnp.concatenate([const_ref[...]] * (WIDTH // LANES), axis=1) + linear

        anchor = jnp.broadcast_to(jnp.sum(const_ref[:8], axis=1, keepdims=True), (8, LANES))
        for ref in (carry_ref, *hv_refs):
            order_loads_after(ref, anchor)

        act, acc = {}, {}
        for d0 in range(0, STREAMS * WIDTH, WIDTH):
            acc[0, d0] = start(carry_ref[:BLK, d0:d0 + WIDTH])
            for i in range(1, LAG):
                vi = carry_ref[BLK * i:BLK * (i + 1), d0:d0 + WIDTH]
                act[(0, d0, *carried[i])] = vi if i <= cfg["act"] else _act(vi)
            write_vpu_operand(0, d0, 0, 7)

        normalized = False
        for kind, *args in events:
            if kind == "v":
                b, d0, blocks = args
                v = hidden_mxu(b, d0, blocks)
                if blocks[0][0] == ntile:
                    acc[b, d0] = start(v[:BLK])
                    v, blocks = v[BLK:], blocks[1:]
                if blocks:
                    g = _act(v)
                    for i, blk in enumerate(blocks):
                        act[(b, d0, *blk)] = g[BLK * i:BLK * (i + 1)]
            elif kind == "y":
                b, d0, js = args
                next_b, next_d0 = divmod(b * D + d0 + STREAMS * WIDTH, D)
                for k, j in enumerate(cfg["spread"]):
                    if j in js and next_b < nb:
                        ref = write_vpu_operand(next_b, next_d0, k, k + 1)
                        order_loads_after(w2t_ref, ref[pl.ds(64 * k + 28 if pitch == 8 else 8 * pitch * k, 8), :])
                for j in js:
                    if (b, d0, j, 7) not in act:
                        act[b, d0, j, 7] = _act(hidden_vpu(b, d0, j))
                g = jnp.concatenate([act.pop((b, d0, j, r)) for j in js for r in range(8)], axis=0)
                acc[b, d0] += _dot(_bf16(w2t_ref[:8, js[0] * LANES:(js[-1] + 1) * LANES]), g)
                if js[-1] == ntile - 1:
                    if cfg["osplit"] and (b, d0) == (nb - 1, 0):
                        assert min(acc)[0] == b
                        output_copy(it * nb, b).start()
                    o_ref[it * nb + b, :, d0:d0 + WIDTH] = (acc.pop((b, d0)) * (0.5 / ALPHA)).astype(o_ref.dtype)
            else:
                if not normalized:
                    var = layernorm(jnp.minimum((it + 1) * nb, B - nb))
                    if cfg["ln_tie"]:
                        order_loads_after(h_refs[0], jnp.broadcast_to(var[-1, 8:], (8, LANES)))
                    normalized = True
                write_carry(*args)
        assert not act and not acc
        if cfg["osplit"]:
            output_copy(it * nb + nb - 1, 1).start()
        else:
            output_copy(it * nb, nb).start()

    output_copy(0, B).wait()


def make(**overrides):
    cfg = dict(CFG, **overrides)

    def kernel(*refs):
        _kernel(cfg, *refs)

    @jax.jit
    def fn(x, w1, b1, w2, b2):
        B, S, D = x.shape
        F = w1.shape[1]
        nb = cfg["step"]
        assert S == BLK and B % nb == 0 and D % (STREAMS * WIDTH) == 0 and F % LANES == 0
        return pl.pallas_call(
            kernel,
            in_specs=[pl.BlockSpec(memory_space=pl.ANY)] * 5,
            out_specs=pl.BlockSpec(memory_space=pl.ANY),
            out_shape=jax.ShapeDtypeStruct((B, S, D), x.dtype),
            scratch_shapes=[
                pltpu.VMEM((S, F), bf16),
                pltpu.VMEM((F,), bf16),
                pltpu.VMEM((S, F), bf16),
                pltpu.VMEM((S,), bf16),
                pltpu.VMEM((B, S, D), x.dtype),
                pltpu.VMEM((B, S, D), x.dtype),
                pltpu.SemaphoreType.DMA((3,)),
                pltpu.VMEM((F // 2 + 8, LANES), i32),
                pltpu.VMEM((8 + 8, F), i32),
                pltpu.VMEM((S, LANES), f32),
                pltpu.VMEM((F // LANES - len(cfg["mxu_only"]), NPROD + 2, 8, LANES), f32),
                pltpu.VMEM((LAG * BLK + 8, STREAMS * WIDTH), f32),
                *[pltpu.VMEM((8 + 8, D), i32)] * nb,
                *[pltpu.VMEM((max(8, cfg['hm']) * NPROD + 8, LANES), f32)] * (nb * D // WIDTH),
            ],
            compiler_params=pltpu.CompilerParams(vmem_limit_bytes=48 * 2**20),
            name="mixer_token_mlp",
        )(x, w1, b1, w2.T, b2)

    return fn


_fn = make(**{})


@jax.jit
def pallas_standalone__mixer_token_mlp__sampling_kernel(x, w1, b1, w2, b2):
    return _fn(x, w1, b1, w2, b2)
```

```python
import jax
import jax.numpy as jnp
import numpy as np
from jax import lax
from jax.experimental import pallas as pl
from jax.experimental.pallas import tpu as pltpu

_C1 = float(np.sqrt(2.0 / np.pi))
ALPHA = (0.044715 * _C1) ** (1.0 / 3.0)
KAPPA = _C1 / ALPHA
ALPHA_HI = 0.328125
LN_EPS = 1e-5

LANES = 128
BLK = 16
WIDTH = 2 * LANES
STREAMS = 2
LAG = 8
NPROD = 7 * 8

FIRST = 2
STEP = 5
MXU_ONLY = (5, 11, 16, 22, 27)
WARMUP = (0, 1, 2)
SPREAD = (4, 26)

f32, bf16, i32 = jnp.float32, jnp.bfloat16, jnp.int32


def _dot(a, b, b_axis=0):
    return lax.dot_general(a, b, (((1,), (b_axis,)), ((), ())), preferred_element_type=f32)


def _iota(shape, axis):
    return lax.broadcasted_iota(i32, shape, axis)


def _words(a):
    return pltpu.bitcast(a, i32)


def _bf16(words):
    return pltpu.bitcast(words, bf16)


def _act(v):
    return v * jnp.tanh(v * (v * v + KAPPA))


def _plan(ntile, nbatch, d, cold):
    passes = [(b, d0) for b in range(nbatch) for d0 in range(0, d, STREAMS * WIDTH)]
    events = []
    for k in range(STREAMS):
        blocks, tiles = [], []
        for p, (b, d0) in enumerate(passes):
            where = (b, d0 + k * WIDTH)
            blocks.append((where, (ntile, 0)))
            for j in range(ntile):
                whole = j in MXU_ONLY or (p == 0 and (cold or j in WARMUP))
                blocks += [(where, (j, r)) for r in range(7 if whole else 6, -1, -1)]
                tiles.append((where, j, len(blocks) + LAG))
        cuts = sorted({0, len(tiles), *range((k + 1) % 2, len(tiles), 2)})
        due = {tiles[hi - 1][2]: tiles[lo:hi] for lo, hi in zip(cuts, cuts[1:])}
        carried = [] if cold else [blk for _, blk in blocks[:LAG]]
        time, run = 0, []
        for i in range(len(carried), len(blocks) + LAG + 1):
            if run and (i in due or i == len(blocks) or blocks[i][0] != run[0][0]):
                events.append((time, k, ("v", *run[0][0], [blk for _, blk in run])))
                time, run = time + len(run), []
            for where in sorted({t[0] for t in due.get(i, [])}):
                js = [t[1] for t in due[i] if t[0] == where]
                events.append((time, k, ("y", *where, js)))
                time += len(js)
            if i < len(blocks):
                run.append(blocks[i])
            elif i == len(blocks):
                events.append((time, k, ("carry", k * WIDTH)))
                time += LAG
    events = [e[2] for e in sorted(events, key=lambda e: e[:2])]
    kinds = [e[0] for e in events]
    assert "v" not in kinds[kinds.index("carry"):]
    return carried, events


def _kernel(x_hbm, w1_hbm, b1_hbm, w2t_hbm, b2_hbm, o_hbm,
            w1_in, b1_in, w2t_in, b2_in, x_ref, o_ref, sems, zero_ref,
            w1t_ref, w2t_ref, const_ref, wv_ref, carry_ref, *h_refs):
    B, S, D = x_ref.shape
    ntile = w1_in.shape[1] // LANES
    h_refs, hv_refs = h_refs[:STEP], h_refs[STEP:]
    vpu_tiles = [j for j in range(ntile) if j not in MXU_ONLY]
    carried, _ = _plan(ntile, STEP, D, False)

    def layernorm(first, n):
        x = x_ref[pl.ds(first, n)].astype(f32)
        xc = x - jnp.sum(x, axis=-1, keepdims=True) * (1.0 / D)
        var = jnp.sum(xc * xc, axis=-1, keepdims=True) * (1.0 / D)
        h = (xc * (ALPHA * lax.rsqrt(var + LN_EPS))).astype(bf16)
        for b in range(n):
            h_refs[b][:8] = _words(h[b])
        return var

    def hidden_mxu(b, d0, blocks):
        h = _bf16(h_refs[b][:8, d0:d0 + WIDTH])
        row = _iota((S, WIDTH), 0)
        one = jnp.where(row == 0, ALPHA_HI, jnp.where(row == 1, ALPHA - ALPHA_HI, 0.0)).astype(bf16)
        w = _bf16(jnp.concatenate([w1t_ref[pl.ds(8 * (8 * j + r), 8), :] for j, r in blocks], axis=0))
        rhs = [h, one, h] if (ntile, 0) in blocks else [h, one]
        return _dot(w[:, :S * len(rhs)], jnp.concatenate(rhs, axis=0))

    def hidden_vpu(b, d0, lo):
        ref = hv_refs[(b * D + d0) // WIDTH]

        def mac(acc, k):
            for n in range(8 * k, 8 * k + 8):
                term = wv_ref[lo:, n] * ref[pl.ds(8 * n, 8), :]
                acc = term if acc is None else acc + term
            return acc

        p5 = mac(None, 4)
        u1 = mac(wv_ref[lo:, NPROD], 0)
        u2 = mac(u1, 5)
        u3 = mac(u2 + wv_ref[lo:, NPROD + 1], 6)
        top = jnp.concatenate([mac(u1, 1), mac(u2 + p5, 2)], axis=2)
        bottom = jnp.concatenate([mac(u3, 3), u3 + p5], axis=2)
        return jnp.concatenate([top, bottom], axis=1)

    def write_vpu_operand(b, d0, lo, hi):
        h = _bf16(h_refs[b][:8, d0:d0 + WIDTH]).astype(f32)
        h11, h12, h21, h22 = h[:8, :LANES], h[:8, LANES:], h[8:, :LANES], h[8:, LANES:]
        t1 = h12 - h11
        t2 = h22 - t1
        factors = [h11, h21, h22, h21 - t2, t1, t2, h22 - h12]
        ref = hv_refs[(b * D + d0) // WIDTH]
        for k, r in (divmod(n, 8) for n in range(lo, hi)):
            ref[pl.ds(64 * k + r, 8, stride=8), :] = factors[k]
        return ref[pl.ds(64 * k + r + 56, 1), :]

    def write_vpu_weights(i, w):
        def column(c):
            col = jnp.broadcast_to(w.astype(f32)[:, c:c + 1], (BLK, LANES))
            return col[:8], col[8:]

        for s in range(8):
            (w11, w21), (w12, w22) = column(s), column(8 + s)
            s1 = w21 + w22
            s2 = s1 - w11
            for k, factor in enumerate([w11, w12, w12 - s2, w22, s1, s2, w11 - w21]):
                wv_ref[i, 8 * k + s] = factor
        bias1, bias2 = column(S)
        wv_ref[i, NPROD] = ALPHA * bias1
        wv_ref[i, NPROD + 1] = ALPHA * (bias2 - bias1)

    def write_weights():
        w1, w2t = w1_in[...], w2t_in[...]
        b1 = b1_in[...].astype(f32).reshape(ntile, LANES)
        bias = [jnp.where(_iota((S, LANES), 0) < 2, b1[j:j + 1], 0.0) for j in range(ntile)]
        bias = jnp.concatenate(bias, axis=1).astype(bf16)
        w2t_ref[:8] = _words(w2t)
        ww = _dot(w2t, jnp.concatenate([w1, bias, w1], axis=0), b_axis=1)
        lane, head = _iota((S, 3 * S), 1), ww.astype(bf16).astype(f32)
        split = jnp.where(lane < S, head, jnp.where(lane < 2 * S, 0.0, ww - head))
        w1t_ref[pl.ds(64 * ntile, 8), :] = _words(split.astype(bf16))
        last_blocks = []
        for j in range(ntile):
            cols = slice(j * LANES, (j + 1) * LANES)
            zeros = jnp.zeros((LANES - 2 * S, LANES), bf16)
            wt = jnp.concatenate([w1_in[:, cols], bias[:, cols], zeros], axis=0).T
            w1t_ref[pl.ds(64 * j, 64), :] = _words(wt[:, :3 * S])
            last_blocks.append(wt[LANES - BLK:])
        for i, j in enumerate(vpu_tiles):
            write_vpu_weights(i, last_blocks[j])
        b2 = jnp.where(_iota((S, S), 0) == _iota((S, S), 1), b2_in[...].astype(f32)[None, :], 0.0)
        const = 0.5 * ww[:, S:S + 1] + jnp.sum(b2, axis=1, keepdims=True)
        const_ref[...] = jnp.broadcast_to(const, (S, LANES))

    def output_copy(first, n):
        rows = pl.ds(first, n)
        return pltpu.make_async_copy(o_ref.at[rows], o_hbm.at[rows], sems.at[2])

    def run(first, nbatch, zero, cold):
        def order_loads_after(ref, value):
            rows = pl.ds(ref.shape[0] - 8 + pl.multiple_of(zero, 8), 8)
            ref[rows, :LANES] = pltpu.bitcast(jnp.broadcast_to(value, (8, LANES)), ref.dtype)

        if cold:
            anchor = layernorm(first, nbatch)[0, :8]
            write_weights()
        else:
            anchor = jnp.sum(const_ref[:8], axis=1, keepdims=True)
        for ref in (carry_ref, *hv_refs[:nbatch * D // WIDTH]):
            order_loads_after(ref, anchor)

        act, acc = {}, {}
        for d0 in range(0, 0 if cold else STREAMS * WIDTH, WIDTH):
            acc[0, d0] = carry_ref[:BLK, d0:d0 + WIDTH]
            for i in range(1, LAG):
                act[(0, d0, *carried[i])] = carry_ref[BLK * i:BLK * (i + 1), d0:d0 + WIDTH]
            write_vpu_operand(0, d0, 0, NPROD)

        normalized = False
        for kind, *args in _plan(ntile, nbatch, D, cold)[1]:
            if kind == "v":
                b, d0, blocks = args
                v = hidden_mxu(b, d0, blocks)
                if blocks[0][0] == ntile:
                    acc[b, d0] = v[:BLK]
                    v, blocks = v[BLK:], blocks[1:]
                if blocks:
                    g = _act(v)
                    for i, blk in enumerate(blocks):
                        act[(b, d0, *blk)] = g[BLK * i:BLK * (i + 1)]
            elif kind == "y":
                b, d0, js = args
                next_b, next_d0 = divmod(b * D + d0 + STREAMS * WIDTH, D)
                j0, j1 = SPREAD
                lo, hi = (NPROD * (min(max(j, j0), j1) - j0) // (j1 - j0) for j in (js[0], js[-1] + 1))
                if lo < hi and next_b < nbatch:
                    written = write_vpu_operand(next_b, next_d0, lo, hi)
                    if not cold:
                        order_loads_after(w2t_ref, written)
                for j in js:
                    if (b, d0, j, 7) not in act:
                        lo = vpu_tiles.index(j)
                        g = _act(hidden_vpu(b, d0, lo))
                        for i, tile in enumerate(vpu_tiles[lo:]):
                            act[b, d0, tile, 7] = g[i]
                g = jnp.concatenate([act.pop((b, d0, j, r)) for j in js for r in range(8)], axis=0)
                acc[b, d0] += _dot(_bf16(w2t_ref[:8, js[0] * LANES:(js[-1] + 1) * LANES]), g)
                if js[-1] == ntile - 1:
                    if (b, d0) == (nbatch - 1, 0):
                        assert min(acc)[0] == b
                        output_copy(first, b).start()
                    const = jnp.concatenate([const_ref[...]] * (WIDTH // LANES), axis=1)
                    y = acc.pop((b, d0)) * (0.5 / ALPHA) + const
                    o_ref[first + b, :, d0:d0 + WIDTH] = y.astype(o_ref.dtype)
            else:
                (d0,) = args
                if not normalized:
                    var = layernorm(jnp.minimum(first + nbatch, B - STEP), STEP)
                    order_loads_after(h_refs[0], var[-1, 8:])
                    normalized = True
                v = hidden_mxu(0, d0, carried)
                for i in range(LAG):
                    vi = v[BLK * i:BLK * (i + 1)]
                    carry_ref[BLK * i:BLK * (i + 1), d0:d0 + WIDTH] = _act(vi) if i else vi
        assert not act and not acc
        output_copy(first + nbatch - 1, 1).start()

    early = FIRST + STEP
    copies = [pltpu.make_async_copy(src, dst, sems.at[0]) for src, dst in [
        (w1_hbm, w1_in), (b1_hbm, b1_in), (w2t_hbm, w2t_in), (b2_hbm, b2_in),
        (x_hbm.at[:early], x_ref.at[:early])]]
    rest_of_x = pltpu.make_async_copy(x_hbm.at[early:], x_ref.at[early:], sems.at[1])
    for copy in (*copies, rest_of_x):
        copy.start()

    @pl.loop(0, 2)
    def _(i):
        zero_ref[i] = 0

    for copy in copies:
        copy.wait()
    run(0, FIRST, zero_ref[1], True)
    rest_of_x.wait()

    @pl.loop(0, (B - FIRST) // STEP)
    def _(it):
        run(FIRST + it * STEP, STEP, (it >> 20) * 8, False)

    output_copy(0, B).wait()


@jax.jit
def pallas_standalone__mixer_token_mlp__sampling_kernel(
    x: jax.Array,
    w1: jax.Array,
    b1: jax.Array,
    w2: jax.Array,
    b2: jax.Array,
):
    B, S, D = x.shape
    F = w1.shape[1]
    assert S == BLK and (B - FIRST) % STEP == 0 and D % (STREAMS * WIDTH) == 0 and F == 28 * LANES
    return pl.pallas_call(
        lambda *refs: _kernel(*refs),
        in_specs=[pl.BlockSpec(memory_space=pl.ANY)] * 5,
        out_specs=pl.BlockSpec(memory_space=pl.ANY),
        out_shape=jax.ShapeDtypeStruct((B, S, D), x.dtype),
        scratch_shapes=[
            pltpu.VMEM((S, F), bf16),
            pltpu.VMEM((F,), bf16),
            pltpu.VMEM((S, F), bf16),
            pltpu.VMEM((S,), bf16),
            pltpu.VMEM((B, S, D), x.dtype),
            pltpu.VMEM((B, S, D), x.dtype),
            pltpu.SemaphoreType.DMA((3,)),
            pltpu.SMEM((2,), i32),
            pltpu.VMEM((F // 2 + 8, 3 * S), i32),
            pltpu.VMEM((8 + 8, F), i32),
            pltpu.VMEM((S, LANES), f32),
            pltpu.VMEM((F // LANES - len(MXU_ONLY), NPROD + 2, 8, LANES), f32),
            pltpu.VMEM((LAG * BLK + 8, STREAMS * WIDTH), f32),
            *[pltpu.VMEM((8 + 8, D), i32)] * STEP,
            *[pltpu.VMEM((8 * NPROD + 8, LANES), f32)] * (STEP * D // WIDTH),
        ],
        compiler_params=pltpu.CompilerParams(vmem_limit_bytes=48 * 2**20),
        name="mixer_token_mlp",
    )(x, w1, b1, w2.T, b2)
```

```python
import jax
import jax.numpy as jnp
import numpy as np
from jax import lax
from jax.experimental import pallas as pl
from jax.experimental.pallas import tpu as pltpu

_C1 = float(np.sqrt(2.0 / np.pi))
ALPHA = (0.044715 * _C1) ** (1.0 / 3.0)
KAPPA = _C1 / ALPHA
ALPHA_HI = 0.328125
LN_EPS = 1e-5

LANES = 128
BLK = 16
WIDTH = 2 * LANES
STREAMS = 2
LAG = 8
NPROD = 7 * 8

FIRST = 2
STEP = 5
MXU_ONLY = (5, 11, 16, 22, 27)
WARMUP = (0, 1, 2)
SPREAD = (4, 26)

f32, bf16, i32 = jnp.float32, jnp.bfloat16, jnp.int32


def _dot(a, b, b_axis=0):
    return lax.dot_general(a, b, (((1,), (b_axis,)), ((), ())), preferred_element_type=f32)


def _iota(shape, axis):
    return lax.broadcasted_iota(i32, shape, axis)


def _words(a):
    return pltpu.bitcast(a, i32)


def _bf16(words):
    return pltpu.bitcast(words, bf16)


def _act(v):
    return v * jnp.tanh(v * (v * v + KAPPA))


def _plan(ntile, nbatch, d, cold):
    passes = [(b, d0) for b in range(nbatch) for d0 in range(0, d, STREAMS * WIDTH)]
    events = []
    for k in range(STREAMS):
        blocks, tiles = [], []
        for p, (b, d0) in enumerate(passes):
            where = (b, d0 + k * WIDTH)
            blocks.append((where, (ntile, 0)))
            for j in range(ntile):
                whole = j in MXU_ONLY or (p == 0 and (cold or j in WARMUP))
                blocks += [(where, (j, r)) for r in range(7 if whole else 6, -1, -1)]
                tiles.append((where, j, len(blocks) + LAG))
        cuts = sorted({0, len(tiles), *range((k + 1) % 2, len(tiles), 2)})
        due = {tiles[hi - 1][2]: tiles[lo:hi] for lo, hi in zip(cuts, cuts[1:])}
        carried = [] if cold else [blk for _, blk in blocks[:LAG]]
        time, run = 0, []
        for i in range(len(carried), len(blocks) + LAG + 1):
            if run and (i in due or i == len(blocks) or blocks[i][0] != run[0][0]):
                events.append((time, k, ("v", *run[0][0], [blk for _, blk in run])))
                time, run = time + len(run), []
            for where in sorted({t[0] for t in due.get(i, [])}):
                js = [t[1] for t in due[i] if t[0] == where]
                events.append((time, k, ("y", *where, js)))
                time += len(js)
            if i < len(blocks):
                run.append(blocks[i])
            elif i == len(blocks):
                events.append((time, k, ("carry", k * WIDTH)))
                time += LAG
    events = [e[2] for e in sorted(events, key=lambda e: e[:2])]
    kinds = [e[0] for e in events]
    assert "v" not in kinds[kinds.index("carry"):]
    return carried, events


def _kernel(x_hbm, w1_hbm, b1_hbm, w2t_hbm, b2_hbm, o_hbm,
            w1_in, b1_in, w2t_in, b2_in, x_ref, o_ref, sems, zero_ref,
            w1t_ref, w2t_ref, const_ref, wv_ref, carry_ref, *h_refs):
    B, S, D = x_ref.shape
    ntile = w1_in.shape[1] // LANES
    h_refs, hv_refs = h_refs[:STEP], h_refs[STEP:]
    vpu_tiles = [j for j in range(ntile) if j not in MXU_ONLY]
    carried, _ = _plan(ntile, STEP, D, False)

    def layernorm(first, n):
        x = x_ref[pl.ds(first, n)].astype(f32)
        xc = x - jnp.sum(x, axis=-1, keepdims=True) * (1.0 / D)
        var = jnp.sum(xc * xc, axis=-1, keepdims=True) * (1.0 / D)
        h = (xc * (ALPHA * lax.rsqrt(var + LN_EPS))).astype(bf16)
        for b in range(n):
            h_refs[b][:8] = _words(h[b])
        return var

    def bias_rows(width):
        row = _iota((S, width), 0)
        return jnp.where(row == 0, ALPHA_HI, jnp.where(row == 1, ALPHA - ALPHA_HI, 0.0)).astype(bf16)

    def b2_column():
        b2 = jnp.where(_iota((S, S), 0) == _iota((S, S), 1), b2_in[...].astype(f32)[None, :], 0.0)
        return jnp.sum(b2, axis=1, keepdims=True)

    def hidden_mxu(b, d0, blocks):
        h, one = _bf16(h_refs[b][:8, d0:d0 + WIDTH]), bias_rows(WIDTH)
        w = _bf16(jnp.concatenate([w1t_ref[pl.ds(8 * (8 * j + r), 8), :] for j, r in blocks], axis=0))
        rhs = [h, one, h] if (ntile, 0) in blocks else [h, one]
        return _dot(w[:, :S * len(rhs)], jnp.concatenate(rhs, axis=0))

    def hidden_vpu(b, d0, lo):
        ref = hv_refs[(b * D + d0) // WIDTH]

        def mac(acc, k):
            for n in range(8 * k, 8 * k + 8):
                term = wv_ref[lo:, n] * ref[pl.ds(8 * n, 8), :]
                acc = term if acc is None else acc + term
            return acc

        p5 = mac(None, 4)
        u1 = mac(wv_ref[lo:, NPROD], 0)
        u2 = mac(u1, 5)
        u3 = mac(u2 + wv_ref[lo:, NPROD + 1], 6)
        top = jnp.concatenate([mac(u1, 1), mac(u2 + p5, 2)], axis=2)
        bottom = jnp.concatenate([mac(u3, 3), u3 + p5], axis=2)
        return jnp.concatenate([top, bottom], axis=1)

    def write_vpu_operand(b, d0, lo, hi):
        h = _bf16(h_refs[b][:8, d0:d0 + WIDTH]).astype(f32)
        h11, h12, h21, h22 = h[:8, :LANES], h[:8, LANES:], h[8:, :LANES], h[8:, LANES:]
        t1 = h12 - h11
        t2 = h22 - t1
        factors = [h11, h21, h22, h21 - t2, t1, t2, h22 - h12]
        ref = hv_refs[(b * D + d0) // WIDTH]
        for k, r in (divmod(n, 8) for n in range(lo, hi)):
            ref[pl.ds(64 * k + r, 8, stride=8), :] = factors[k]
        return ref[pl.ds(64 * k + r + 56, 1), :]

    def write_vpu_weights(i, w):
        left = w.astype(f32)
        right = pltpu.roll(left, LANES - 8, 1)
        s3 = left[:8] - left[8:]
        s4 = right[:8] - (left[8:] + right[8:] - left[:8])

        def column(a, c):
            return jnp.broadcast_to(a[:, c:c + 1], a.shape)

        for s in range(8):
            a, b = column(left, s), column(right, s)
            s1 = a[8:] + b[8:]
            s2 = s1 - a[:8]
            for k, factor in enumerate([a[:8], b[:8], column(s4, s), b[8:], s1, s2, column(s3, s)]):
                wv_ref[i, 8 * k + s] = factor
        bias = column(left, S)
        wv_ref[i, NPROD] = ALPHA * bias[:8]
        wv_ref[i, NPROD + 1] = ALPHA * (bias[8:] - bias[:8])

    def write_weights():
        w1, w2t = w1_in[...], w2t_in[...]
        b1 = b1_in[...].astype(f32).reshape(ntile, LANES)
        bias = [jnp.where(_iota((S, LANES), 0) < 2, b1[j:j + 1], 0.0) for j in range(ntile)]
        bias = jnp.concatenate(bias, axis=1).astype(bf16)
        w2t_ref[:8] = _words(w2t)
        ww = _dot(w2t, jnp.concatenate([w1, bias, w1], axis=0), b_axis=1)
        lane, head = _iota((S, 3 * S), 1), ww.astype(bf16).astype(f32)
        split = jnp.where(lane < S, head, jnp.where(lane < 2 * S, 0.0, ww - head))
        w1t_ref[pl.ds(64 * ntile, 8), :] = _words(split.astype(bf16))
        last_blocks = []
        for j in range(ntile):
            cols = slice(j * LANES, (j + 1) * LANES)
            zeros = jnp.zeros((LANES - 2 * S, LANES), bf16)
            wt = jnp.concatenate([w1_in[:, cols], bias[:, cols], zeros], axis=0).T
            w1t_ref[pl.ds(64 * j, 64), :] = _words(wt[:, :3 * S])
            last_blocks.append(wt[LANES - BLK:])
        for i, j in enumerate(vpu_tiles):
            write_vpu_weights(i, last_blocks[j])
        const_ref[...] = jnp.broadcast_to(0.5 * ww[:, S:S + 1] + b2_column(), (S, LANES))

    def output_copy(first, n):
        rows = pl.ds(first, n)
        return pltpu.make_async_copy(o_ref.at[rows], o_hbm.at[rows], sems.at[2])

    def run(first, nbatch, zero, cold):
        def order_loads_after(ref, value):
            rows = pl.ds(ref.shape[0] - 8 + pl.multiple_of(zero, 8), 8)
            ref[rows, :LANES] = pltpu.bitcast(jnp.broadcast_to(value, (8, LANES)), ref.dtype)

        if cold:
            anchor = layernorm(first, nbatch)[0, :8]
            write_weights()
        else:
            anchor = jnp.sum(const_ref[:8], axis=1, keepdims=True)
        for ref in (carry_ref, *hv_refs[:nbatch * D // WIDTH]):
            order_loads_after(ref, anchor)

        act, acc = {}, {}
        for d0 in range(0, 0 if cold else STREAMS * WIDTH, WIDTH):
            acc[0, d0] = carry_ref[:BLK, d0:d0 + WIDTH]
            for i in range(1, LAG):
                act[(0, d0, *carried[i])] = carry_ref[BLK * i:BLK * (i + 1), d0:d0 + WIDTH]
            write_vpu_operand(0, d0, 0, NPROD)

        normalized = False
        for kind, *args in _plan(ntile, nbatch, D, cold)[1]:
            if kind == "v":
                b, d0, blocks = args
                v = hidden_mxu(b, d0, blocks)
                if blocks[0][0] == ntile:
                    acc[b, d0] = v[:BLK]
                    v, blocks = v[BLK:], blocks[1:]
                if blocks:
                    g = _act(v)
                    for i, blk in enumerate(blocks):
                        act[(b, d0, *blk)] = g[BLK * i:BLK * (i + 1)]
            elif kind == "y":
                b, d0, js = args
                next_b, next_d0 = divmod(b * D + d0 + STREAMS * WIDTH, D)
                j0, j1 = SPREAD
                lo, hi = (NPROD * (min(max(j, j0), j1) - j0) // (j1 - j0) for j in (js[0], js[-1] + 1))
                if lo < hi and next_b < nbatch:
                    written = write_vpu_operand(next_b, next_d0, lo, hi)
                    if not cold:
                        order_loads_after(w2t_ref, written)
                for j in js:
                    if (b, d0, j, 7) not in act:
                        lo = vpu_tiles.index(j)
                        g = _act(hidden_vpu(b, d0, lo))
                        for i, tile in enumerate(vpu_tiles[lo:]):
                            act[b, d0, tile, 7] = g[i]
                g = jnp.concatenate([act.pop((b, d0, j, r)) for j in js for r in range(8)], axis=0)
                acc[b, d0] += _dot(_bf16(w2t_ref[:8, js[0] * LANES:(js[-1] + 1) * LANES]), g)
                if js[-1] == ntile - 1:
                    if (b, d0) == (nbatch - 1, 0):
                        assert min(acc)[0] == b
                        output_copy(first, b).start()
                    const = jnp.concatenate([const_ref[...]] * (WIDTH // LANES), axis=1)
                    y = acc.pop((b, d0)) * (0.5 / ALPHA) + const
                    o_ref[first + b, :, d0:d0 + WIDTH] = y.astype(o_ref.dtype)
            else:
                (d0,) = args
                if not normalized:
                    var = layernorm(jnp.minimum(first + nbatch, B - STEP), STEP)
                    order_loads_after(h_refs[0], var[-1, 8:])
                    normalized = True
                v = hidden_mxu(0, d0, carried)
                for i in range(LAG):
                    vi = v[BLK * i:BLK * (i + 1)]
                    carry_ref[BLK * i:BLK * (i + 1), d0:d0 + WIDTH] = _act(vi) if i else vi
        assert not act and not acc
        output_copy(first + nbatch - 1, 1).start()

    early = FIRST + STEP
    copies = [pltpu.make_async_copy(src, dst, sems.at[0]) for src, dst in [
        (w1_hbm, w1_in), (b1_hbm, b1_in), (w2t_hbm, w2t_in), (b2_hbm, b2_in),
        (x_hbm.at[:early], x_ref.at[:early])]]
    rest_of_x = pltpu.make_async_copy(x_hbm.at[early:], x_ref.at[early:], sems.at[1])
    for copy in (*copies, rest_of_x):
        copy.start()

    @pl.loop(0, 2)
    def _(i):
        zero_ref[i] = 0

    for copy in copies:
        copy.wait()
    run(0, FIRST, zero_ref[1], True)
    rest_of_x.wait()

    @pl.loop(0, (B - FIRST) // STEP)
    def _(it):
        run(FIRST + it * STEP, STEP, (it >> 20) * 8, False)

    may_cancel = jnp.min(b1_in[...].astype(f32).reshape(ntile, LANES)) < -1.0
    output_copy(0, B).wait()

    @pl.when(may_cancel)
    def _():
        @pl.loop(0, B)
        def _(b):
            layernorm(b, 1)

            def tile(j, acc):
                w = _bf16(w1t_ref[pl.ds(pl.multiple_of(64 * j, 64), 64), :])
                v = _dot(w[:, :2 * S], jnp.concatenate([_bf16(h_refs[0][:8]), bias_rows(D)], axis=0))
                cols = pl.ds(pl.multiple_of(j * LANES, LANES), LANES)
                return acc + _dot(_bf16(w2t_ref[:8, cols]), v + _act(v))

            y = lax.fori_loop(0, ntile, tile, jnp.zeros((S, D), f32)) * (0.5 / ALPHA) + b2_column()
            o_ref[b] = y.astype(o_ref.dtype)

        output_copy(0, B).start()
        output_copy(0, B).wait()


@jax.jit
def pallas_standalone__mixer_token_mlp__sampling_kernel(
    x: jax.Array,
    w1: jax.Array,
    b1: jax.Array,
    w2: jax.Array,
    b2: jax.Array,
):
    B, S, D = x.shape
    F = w1.shape[1]
    assert S == BLK and (B - FIRST) % STEP == 0 and D % (STREAMS * WIDTH) == 0 and F == 28 * LANES
    return pl.pallas_call(
        lambda *refs: _kernel(*refs),
        in_specs=[pl.BlockSpec(memory_space=pl.ANY)] * 5,
        out_specs=pl.BlockSpec(memory_space=pl.ANY),
        out_shape=jax.ShapeDtypeStruct((B, S, D), x.dtype),
        scratch_shapes=[
            pltpu.VMEM((S, F), bf16),
            pltpu.VMEM((F,), bf16),
            pltpu.VMEM((S, F), bf16),
            pltpu.VMEM((S,), bf16),
            pltpu.VMEM((B, S, D), x.dtype),
            pltpu.VMEM((B, S, D), x.dtype),
            pltpu.SemaphoreType.DMA((3,)),
            pltpu.SMEM((2,), i32),
            pltpu.VMEM((F // 2 + 8, 3 * S), i32),
            pltpu.VMEM((8 + 8, F), i32),
            pltpu.VMEM((S, LANES), f32),
            pltpu.VMEM((F // LANES - len(MXU_ONLY), NPROD + 2, 8, LANES), f32),
            pltpu.VMEM((LAG * BLK + 8, STREAMS * WIDTH), f32),
            *[pltpu.VMEM((8 + 8, D), i32)] * STEP,
            *[pltpu.VMEM((8 * NPROD + 8, LANES), f32)] * (STEP * D // WIDTH),
        ],
        compiler_params=pltpu.CompilerParams(vmem_limit_bytes=48 * 2**20),
        name="mixer_token_mlp",
    )(x, w1, b1, w2.T, b2)
```
